```python
import os as _os
_os.environ.setdefault("JAX_PLATFORMS", "cpu")
import jax
import jax.numpy as jnp

def _softmax(x, axis=-1):
    return jax.nn.softmax(x, axis=axis)
def _gelu(x):
    return jax.nn.gelu(x, approximate=True)
def _silu(x):
    return jax.nn.silu(x)
def _sigmoid(x):
    return jax.nn.sigmoid(x)
def _layernorm(x, axis=-1, eps=1e-5):
    m = jnp.mean(x, axis=axis, keepdims=True)
    v = jnp.var(x, axis=axis, keepdims=True)
    return (x - m) / jnp.sqrt(v + eps)
def _scatter_add(tgt, idx, src, axis=0):
    return tgt.at[idx].add(src)
def _segment_sum(src, seg, n):
    return jax.ops.segment_sum(src, seg, n)
class _Rng:
    def __init__(self, key):
        self._k = key
    def _next(self):
        self._k, sub = jax.random.split(self._k)
        return sub
    def normal(self, shape):
        return jax.random.normal(self._next(), shape, dtype=jnp.bfloat16)
    def randint(self, lo, hi, shape):
        return jax.random.randint(self._next(), shape, lo, hi, dtype=jnp.int32)
    def uniform(self, shape, lo=0.0, hi=1.0):
        return jax.random.uniform(self._next(), shape, jnp.bfloat16, lo, hi)
    def permutation(self, n):
        return jax.random.permutation(self._next(), n)


kernel_name = 'gated_mix__gqa_block_cached__dense_activation_squared_relu__decode'

def setup_inputs():
    _rng = _Rng(jax.random.key(int.from_bytes(__import__("os").urandom(4), "little")))
    _w = (lambda a: (lambda t: t.astype(jnp.bfloat16) if jnp.issubdtype(t.dtype, jnp.floating) else t)(jnp.asarray(a)))
    def _A_setup():
        B, Sq, D = 4, 1, 512
        Hq, Hkv, Sk, Dh = 32, 8, 4096, 128
        assert Hq % Hkv == 0, (Hq, Hkv)
        return {
            "x": _w((lambda *s: _rng.normal(s) * 0.05)(B, Sq, D)),
            "k_cache": _w((lambda *s: _rng.normal(s) * 3.2)(B, Hkv, Sk, Dh)),
            "v_cache": _w((lambda *s: _rng.normal(s) * 1.6)(B, Hkv, Sk, Dh)),
            "wq": _w((lambda *s: _rng.normal(s) * 3.2)(D, Hq * Dh) * (D ** -0.5)),
            "wo": _w((lambda *s: _rng.normal(s) * 1.6)(Hq * Dh, D) * ((Hq * Dh) ** -0.5)),
        }
    _A_in = _A_setup()

    def _B_setup():
        B, S, D, F = 4, 1, 512, 1792
        return {
            "x": _w((lambda *s: _rng.normal(s) * 0.05)(B, S, D)),
            "w1": _w((lambda *s: _rng.normal(s) * 0.1)(D, F)),
            "b1": _w((lambda *s: _rng.normal(s) * 0.05)(F)),
            "w2": _w((lambda *s: _rng.normal(s) * 0.05)(F, D)),
            "b2": _w((lambda *s: _rng.normal(s) * 0.05)(D)),
        }
    _B_in = _B_setup()

    return {
        "A_x": _A_in["x"],
        "A_k_cache": _A_in["k_cache"],
        "A_v_cache": _A_in["v_cache"],
        "A_wq": _A_in["wq"],
        "A_wo": _A_in["wo"],
        "B_x": _B_in["x"],
        "B_w1": _B_in["w1"],
        "B_b1": _B_in["b1"],
        "B_w2": _B_in["w2"],
        "B_b2": _B_in["b2"],
        "gate_w": _w((lambda *s: _rng.normal(s) * 0.05)(512) * 16.0),
    }

def reference(A_x, A_k_cache, A_v_cache, A_wq, A_wo, B_x, B_w1, B_b1, B_w2, B_b2, gate_w):
    def _A_ref(x, k_cache, v_cache, wq, wo):
        B, Sq, D = x.shape
        Hq, Dh = 32, 128
        Hkv = k_cache.shape[1]
        rep = Hq // Hkv
        q = (lambda x, *d: x.transpose(*d))((x @ wq).reshape(B, Sq, Hq, Dh), 0, 2, 1, 3)
        k = jnp.repeat(k_cache, rep, axis=1)
        v = jnp.repeat(v_cache, rep, axis=1)
        scores = jnp.einsum("bhqd,bhkd->bhqk", q, k) * (Dh ** -0.5)
        p = _softmax(scores, axis=-1)
        o = jnp.einsum("bhqk,bhkd->bhqd", p, v)
        return (lambda x, *d: x.transpose(*d))(o, 0, 2, 1, 3).reshape(B, Sq, Hq * Dh) @ wo

    def _B_ref(x, w1, b1, w2, b2):
        h = jnp.einsum("bsd,df->bsf", x, w1) + b1
        zero = jnp.zeros_like(h)
        r = jnp.where(h > zero, h, zero)
        h = r * r
        out = jnp.einsum("bsf,fd->bsd", h, w2) + b2
        return out

    x = A_x
    g = _sigmoid((x * gate_w).sum(-1, keepdims=True))
    a = _A_ref(x, A_k_cache, A_v_cache, A_wq, A_wo)
    b = _B_ref(x, B_w1, B_b1, B_w2, B_b2)
    return g * a + (1 - g) * b
```

```python
import jax
import jax.numpy as jnp
import jax.experimental.pallas as pl
import jax.experimental.pallas.tpu as pltpu


def _make_kernel(B, Hkv, rep, Dh, Sk, D, F, FCH):
    n_fch = F // FCH
    scale = float(Dh) ** -0.5
    f32 = jnp.float32
    bf16 = jnp.bfloat16

    def kernel(x_ref, k_ref, v_ref, wq_ref, wo_ref, w1_ref, b1_ref, w2_ref,
               b2_ref, gw_ref, o_ref, q_scr, oa_scr, acc_scr, ffn_scr):
        h = pl.program_id(0)
        b = pl.program_id(1)
        x = x_ref[...]

        @pl.when(jnp.logical_and(h == 0, b == 0))
        def _init():
            acc_scr[...] = jnp.zeros_like(acc_scr)
            ffn_scr[...] = jnp.zeros_like(ffn_scr)

        @pl.when(b == 0)
        def _qproj():
            q = jnp.dot(x, wq_ref[...], preferred_element_type=f32)
            for bb in range(B):
                for j in range(rep):
                    q_scr[bb, j:j + 1, :] = q[bb:bb + 1, j * Dh:(j + 1) * Dh]

        @pl.when(jnp.logical_and(b == 0, h < n_fch))
        def _ffn():
            hh = jnp.dot(x, w1_ref[...], preferred_element_type=f32)
            hh = hh + b1_ref[...].astype(f32).reshape(1, FCH)
            r = jnp.maximum(hh, 0.0)
            hh = (r * r).astype(bf16)
            ffn_scr[...] += jnp.dot(hh, w2_ref[...], preferred_element_type=f32)

        q = q_scr[b, 0:rep, :].astype(bf16)
        s = jax.lax.dot_general(q, k_ref[...], (((1,), (1,)), ((), ())),
                                preferred_element_type=f32)
        s = s * scale
        m = jnp.max(s, axis=-1, keepdims=True)
        p = jnp.exp(s - m)
        l = jnp.sum(p, axis=-1, keepdims=True)
        o = jnp.dot(p.astype(bf16), v_ref[...], preferred_element_type=f32)
        o = o / l
        oa_scr[b, 0:rep, :] = o

        @pl.when(b == B - 1)
        def _oproj():
            oa = jnp.concatenate([oa_scr[:, j, :] for j in range(rep)], axis=-1)
            acc_scr[...] += jnp.dot(oa.astype(bf16), wo_ref[...],
                                    preferred_element_type=f32)

        @pl.when(jnp.logical_and(h == Hkv - 1, b == B - 1))
        def _fin():
            xf = x.astype(f32)
            g = jax.nn.sigmoid(jnp.sum(xf * gw_ref[...].astype(f32).reshape(1, D), axis=-1,
                                       keepdims=True))
            ffn = ffn_scr[...] + b2_ref[...].astype(f32).reshape(1, D)
            res = g * acc_scr[...] + (1.0 - g) * ffn
            o_ref[...] = res.astype(o_ref.dtype)

    return kernel


@jax.jit
def pallas_gated_mix__gqa_block_cached__dense_activation_squared_relu__decode_kernel(
A_x: jax.Array,
    A_k_cache: jax.Array,
    A_v_cache: jax.Array,
    A_wq: jax.Array,
    A_wo: jax.Array,
    B_x: jax.Array,
    B_w1: jax.Array,
    B_b1: jax.Array,
    B_w2: jax.Array,
    B_b2: jax.Array,
    gate_w: jax.Array,
):
    B, Sq, D = A_x.shape
    _, Hkv, Sk, Dh = A_k_cache.shape
    HqDh = A_wq.shape[1]
    rep = HqDh // (Hkv * Dh)
    F = B_w1.shape[1]
    FCH = 256
    n_fch = F // FCH
    GW = rep * Dh

    kernel = _make_kernel(B, Hkv, rep, Dh, Sk, D, F, FCH)

    def fch(h):
        return jnp.minimum(h, n_fch - 1)

    in_specs = [
        pl.BlockSpec((B, D), lambda h, b: (0, 0)),
        pl.BlockSpec((None, None, Sk, Dh), lambda h, b: (b, h, 0, 0)),
        pl.BlockSpec((None, None, Sk, Dh), lambda h, b: (b, h, 0, 0)),
        pl.BlockSpec((D, GW), lambda h, b: (0, h)),
        pl.BlockSpec((GW, D), lambda h, b: (h, 0)),
        pl.BlockSpec((D, FCH), lambda h, b: (0, fch(h))),
        pl.BlockSpec((FCH,), lambda h, b: (fch(h),)),
        pl.BlockSpec((FCH, D), lambda h, b: (fch(h), 0)),
        pl.BlockSpec((D,), lambda h, b: (0,)),
        pl.BlockSpec((D,), lambda h, b: (0,)),
    ]
    out_spec = pl.BlockSpec((B, D), lambda h, b: (0, 0))

    return pl.pallas_call(
        kernel,
        grid=(Hkv, B),
        in_specs=in_specs,
        out_specs=out_spec,
        out_shape=jax.ShapeDtypeStruct((B, D), A_x.dtype),
        scratch_shapes=[
            pltpu.VMEM((B, 8, Dh), jnp.float32),
            pltpu.VMEM((B, 8, Dh), jnp.float32),
            pltpu.VMEM((B, D), jnp.float32),
            pltpu.VMEM((B, D), jnp.float32),
        ],
        compiler_params=pltpu.CompilerParams(
            dimension_semantics=("arbitrary", "arbitrary"),
            vmem_limit_bytes=64 * 1024 * 1024,
        ),
    )(A_x.reshape(B, D), A_k_cache, A_v_cache, A_wq, A_wo, B_w1, B_b1, B_w2,
      B_b2, gate_w).reshape(B, Sq, D)
```

```python
import jax
import jax.numpy as jnp
import jax.experimental.pallas as pl
import jax.experimental.pallas.tpu as pltpu


def _ffn_schedule(F, n_steps):
    last = n_steps - 1
    tail = [256, 256, 128, 128]
    head_total = F - sum(tail)
    assert head_total >= 0 and head_total % 128 == 0
    head = []
    while head_total > 0:
        c = min(512, head_total)
        head.append(c)
        head_total -= c
    sched = []
    off = 0
    for i, c in enumerate(head):
        sched.append((off, c, 4 * i, 4 * i + 3))
        off += c
    for c in tail:
        sched.append((off, c, last - 1, last))
        off += c
    assert off == F
    return sched


def _make_kernel(B, Hkv, rep, Dh, Sk, D, F):
    scale = float(Dh) ** -0.5
    f32 = jnp.float32
    bf16 = jnp.bfloat16
    n_steps = Hkv * B
    sched = _ffn_schedule(F, n_steps)

    def kernel(x_ref, k_ref, v_ref, wq_ref, wo_ref, w1_hbm, b1_ref, w2_hbm,
               b2_ref, gw_ref, o_ref, q_scr, oa_scr, acc_scr, ffn_scr,
               w1_buf, w2_buf, sem):
        h = pl.program_id(0)
        b = pl.program_id(1)
        step = h * B + b
        x = x_ref[...]

        def w1_copy(ci):
            off, sz, _, _ = sched[ci]
            return pltpu.make_async_copy(w1_hbm.at[:, pl.ds(off, sz)],
                                         w1_buf.at[:, pl.ds(off, sz)],
                                         sem.at[0, ci])

        def w2_copy(ci):
            off, sz, _, _ = sched[ci]
            return pltpu.make_async_copy(w2_hbm.at[pl.ds(off, sz), :],
                                         w2_buf.at[pl.ds(off, sz), :],
                                         sem.at[1, ci])

        def issue(s):
            for ci in range(len(sched)):
                if sched[ci][2] == s:
                    w1_copy(ci).start()
                    w2_copy(ci).start()

        def ffn_chunk(ci):
            off, sz, _, _ = sched[ci]
            w1_copy(ci).wait()
            w2_copy(ci).wait()
            b1 = b1_ref[...].astype(f32).reshape(1, F)[:, off:off + sz]
            hh = jnp.dot(x, w1_buf[:, off:off + sz], preferred_element_type=f32)
            hh = hh + b1
            r = jnp.maximum(hh, 0.0)
            hh = (r * r).astype(bf16)
            ffn_scr[...] += jnp.dot(hh, w2_buf[off:off + sz, :],
                                    preferred_element_type=f32)

        @pl.when(step == 0)
        def _init():
            acc_scr[...] = jnp.zeros_like(acc_scr)
            ffn_scr[...] = jnp.zeros_like(ffn_scr)
            issue(0)

        @pl.when(b == 0)
        def _qproj():
            q = jnp.dot(x, wq_ref[...], preferred_element_type=f32)
            for bb in range(B):
                for j in range(rep):
                    q_scr[bb, j:j + 1, :] = q[bb:bb + 1, j * Dh:(j + 1) * Dh]

        q = q_scr[b, 0:rep, :].astype(bf16)
        s = jax.lax.dot_general(q, k_ref[...], (((1,), (1,)), ((), ())),
                                preferred_element_type=f32)
        s = s * scale
        m = jnp.max(s, axis=-1, keepdims=True)
        p = jnp.exp(s - m)
        l = jnp.sum(p, axis=-1, keepdims=True)
        o = jnp.dot(p.astype(bf16), v_ref[...], preferred_element_type=f32)
        o = o / l
        oa_scr[b, 0:rep, :] = o

        @pl.when(b == B - 1)
        def _oproj():
            oa = jnp.concatenate([oa_scr[:, j, :] for j in range(rep)], axis=-1)
            acc_scr[...] += jnp.dot(oa.astype(bf16), wo_ref[...],
                                    preferred_element_type=f32)

        for s_ in sorted({c[2] for c in sched} | {c[3] for c in sched}):
            @pl.when(step == s_)
            def _(s_=s_):
                for ci in range(len(sched)):
                    if sched[ci][3] == s_:
                        ffn_chunk(ci)
                if s_ != 0:
                    issue(s_)

        @pl.when(step == n_steps - 1)
        def _fin():
            xf = x.astype(f32)
            g = jax.nn.sigmoid(jnp.sum(xf * gw_ref[...].astype(f32).reshape(1, D),
                                       axis=-1, keepdims=True))
            ffn = ffn_scr[...] + b2_ref[...].astype(f32).reshape(1, D)
            res = g * acc_scr[...] + (1.0 - g) * ffn
            o_ref[...] = res.astype(o_ref.dtype)

    return kernel, len(sched)


@jax.jit
def pallas_gated_mix__gqa_block_cached__dense_activation_squared_relu__decode_kernel(
A_x: jax.Array,
    A_k_cache: jax.Array,
    A_v_cache: jax.Array,
    A_wq: jax.Array,
    A_wo: jax.Array,
    B_x: jax.Array,
    B_w1: jax.Array,
    B_b1: jax.Array,
    B_w2: jax.Array,
    B_b2: jax.Array,
    gate_w: jax.Array,
):
    B, Sq, D = A_x.shape
    _, Hkv, Sk, Dh = A_k_cache.shape
    HqDh = A_wq.shape[1]
    rep = HqDh // (Hkv * Dh)
    F = B_w1.shape[1]
    GW = rep * Dh

    kernel, n_chunks = _make_kernel(B, Hkv, rep, Dh, Sk, D, F)

    in_specs = [
        pl.BlockSpec((B, D), lambda h, b: (0, 0)),
        pl.BlockSpec((None, None, Sk, Dh), lambda h, b: (b, h, 0, 0)),
        pl.BlockSpec((None, None, Sk, Dh), lambda h, b: (b, h, 0, 0)),
        pl.BlockSpec((D, GW), lambda h, b: (0, h)),
        pl.BlockSpec((GW, D), lambda h, b: (h, 0)),
        pl.BlockSpec(memory_space=pl.ANY),
        pl.BlockSpec((F,), lambda h, b: (0,)),
        pl.BlockSpec(memory_space=pl.ANY),
        pl.BlockSpec((D,), lambda h, b: (0,)),
        pl.BlockSpec((D,), lambda h, b: (0,)),
    ]
    out_spec = pl.BlockSpec((B, D), lambda h, b: (0, 0))

    return pl.pallas_call(
        kernel,
        grid=(Hkv, B),
        in_specs=in_specs,
        out_specs=out_spec,
        out_shape=jax.ShapeDtypeStruct((B, D), A_x.dtype),
        scratch_shapes=[
            pltpu.VMEM((B, 8, Dh), jnp.float32),
            pltpu.VMEM((B, 8, Dh), jnp.float32),
            pltpu.VMEM((B, D), jnp.float32),
            pltpu.VMEM((B, D), jnp.float32),
            pltpu.VMEM((D, F), B_w1.dtype),
            pltpu.VMEM((F, D), B_w2.dtype),
            pltpu.SemaphoreType.DMA((2, n_chunks)),
        ],
        compiler_params=pltpu.CompilerParams(
            dimension_semantics=("arbitrary", "arbitrary"),
            vmem_limit_bytes=64 * 1024 * 1024,
        ),
    )(A_x.reshape(B, D), A_k_cache, A_v_cache, A_wq, A_wo, B_w1, B_b1, B_w2,
      B_b2, gate_w).reshape(B, Sq, D)
```
